```python
import jax
import jax.numpy as jnp

def _softmax(x, axis=-1):
    return jax.nn.softmax(x, axis=axis)
def _gelu(x):
    return jax.nn.gelu(x, approximate=True)
def _silu(x):
    return jax.nn.silu(x)
def _sigmoid(x):
    return jax.nn.sigmoid(x)
def _layernorm(x, axis=-1, eps=1e-5):
    m = jnp.mean(x, axis=axis, keepdims=True)
    v = jnp.var(x, axis=axis, keepdims=True)
    return (x - m) / jnp.sqrt(v + eps)
def _scatter_add(tgt, idx, src, axis=0):
    return tgt.at[idx].add(src)
def _segment_sum(src, seg, n):
    return jax.ops.segment_sum(src, seg, n)
class _Rng:
    def __init__(self, key):
        self._k = key
    def _next(self):
        self._k, sub = jax.random.split(self._k)
        return sub
    def normal(self, shape):
        return jax.random.normal(self._next(), shape, dtype=jnp.bfloat16)
    def randint(self, lo, hi, shape):
        return jax.random.randint(self._next(), shape, lo, hi, dtype=jnp.int32)
    def uniform(self, shape, lo=0.0, hi=1.0):
        return jax.random.uniform(self._next(), shape, jnp.bfloat16, lo, hi)
    def permutation(self, n):
        return jax.random.permutation(self._next(), n)


kernel_name = 'sequential_preLN__mha_block_cached__moe_arch_mod__decode'

def setup_inputs():
    _rng = _Rng(jax.random.key(int.from_bytes(__import__("os").urandom(4), "little")))
    _w = (lambda a: (lambda t: t.astype(jnp.bfloat16) if jnp.issubdtype(t.dtype, jnp.floating) else t)(jnp.asarray(a)))
    def _A_setup():
        B, Sq, D = 4, 1, 640
        H, Sk, Dh = 32, 8192, 192
        return {
            "x": _w((lambda *s: _rng.normal(s) * 0.05)(B, Sq, D)),
            "k_cache": _w((lambda *s: _rng.normal(s) * 0.05)(B, H, Sk, Dh)),
            "v_cache": _w((lambda *s: _rng.normal(s) * 0.05)(B, H, Sk, Dh)),
            "wq": _w((lambda *s: _rng.normal(s) * 0.05)(D, H * Dh) * (D ** -0.5)),
            "wo": _w((lambda *s: _rng.normal(s) * 0.05)(H * Dh, D) * ((H * Dh) ** -0.5)),
        }
    _A_in = _A_setup()

    def _B_setup():
        B, S, D, F, C = 4, 1, 640, 1536, 1
        return {
            "x": _w((lambda *s: _rng.normal(s) * 0.05)(B, S, D)),
            "w_r": _w((lambda *s: _rng.normal(s) * 0.05)(D)),
            "w_gate": _w((lambda *s: _rng.normal(s) * 0.05)(D, F)),
            "w_up": _w((lambda *s: _rng.normal(s) * 0.05)(D, F)),
            "w_down": _w((lambda *s: _rng.normal(s) * 0.05)(F, D)),
        }
    _B_in = _B_setup()

    return {
        "A_x": _A_in["x"],
        "A_k_cache": _A_in["k_cache"],
        "A_v_cache": _A_in["v_cache"],
        "A_wq": _A_in["wq"],
        "A_wo": _A_in["wo"],
        "B_x": _B_in["x"],
        "B_w_r": _B_in["w_r"],
        "B_w_gate": _B_in["w_gate"],
        "B_w_up": _B_in["w_up"],
        "B_w_down": _B_in["w_down"],
    }

def reference(A_x, A_k_cache, A_v_cache, A_wq, A_wo, B_x, B_w_r, B_w_gate, B_w_up, B_w_down):
    def _A_ref(x, k_cache, v_cache, wq, wo):
        B, Sq, D = x.shape
        H, Dh = 32, 192
        q = (lambda x, *d: x.transpose(*d))((x @ wq).reshape(B, Sq, H, Dh), 0, 2, 1, 3)
        scores = jnp.einsum("bhqd,bhkd->bhqk", q, k_cache) * (Dh ** -0.5)
        p = _softmax(scores, axis=-1)
        o = jnp.einsum("bhqk,bhkd->bhqd", p, v_cache)
        return (lambda x, *d: x.transpose(*d))(o, 0, 2, 1, 3).reshape(B, Sq, H * Dh) @ wo

    def _B_ref(x, w_r, w_gate, w_up, w_down):
        B, S, D = x.shape
        C = 1
        r = x @ w_r
        idx = jnp.argsort(-r, axis=-1)[:, :C]
        idx_e = jnp.repeat(idx.reshape(B, C, 1), D, axis=2)
        x_sel = jnp.take_along_axis(x, idx_e, axis=1)
        g = _silu(x_sel @ w_gate)
        u = x_sel @ w_up
        y = (g * u) @ w_down
        r_sel = _sigmoid(jnp.take_along_axis(r, idx, axis=1))
        y = y * r_sel.reshape(B, C, 1)
        b_off = (jnp.arange(B) * S).reshape(B, 1)
        flat_idx = (idx + b_off).reshape(B * C)
        zero = (x * 0.0).reshape(B * S, D)
        upd = _scatter_add(zero, flat_idx, y.reshape(B * C, D), axis=0)
        return x + upd.reshape(B, S, D)

    x = A_x
    h = x + _A_ref(_layernorm(x, axis=-1), A_k_cache, A_v_cache, A_wq, A_wo)
    h2 = h + _B_ref(_layernorm(h, axis=-1), B_w_r, B_w_gate, B_w_up, B_w_down)
    return h2
```

```python
import jax
import jax.numpy as jnp
import jax.experimental.pallas as pl
import jax.experimental.pallas.tpu as pltpu

_B, _H, _DH, _S, _D, _F = 4, 32, 192, 8192, 640, 1536
_NPAIR = 2
_FC = 4
_EPS = 1e-5


def _layernorm(x):
    m = jnp.mean(x, axis=-1, keepdims=True)
    c = x - m
    v = jnp.mean(c * c, axis=-1, keepdims=True)
    return c / jnp.sqrt(v + _EPS)


def _kernel(x_hbm, kt_hbm, vt_hbm, wq_hbm, wo_hbm, wr_hbm, wg_hbm, wu_hbm, wd_hbm,
            o_ref,
            x_v, wq_v, wo_v, wr_v, wg_v, wu_v, wd_v, k_ring, v_ring, q_s,
            k_sem, v_sem, w_sem, d_sem):
    f32, bf16 = jnp.float32, jnp.bfloat16
    n = _B * _H
    fc = _F // _FC

    def kv_copy(src, ring, sem, i):
        slot = i % _NPAIR
        return pltpu.make_async_copy(src.at[i % _B, i // _B], ring.at[slot], sem.at[slot])

    cp_wq = pltpu.make_async_copy(wq_hbm, wq_v, w_sem.at[0])
    cp_x = pltpu.make_async_copy(x_hbm, x_v, w_sem.at[1])
    cp_wr = pltpu.make_async_copy(wr_hbm, wr_v, w_sem.at[2])
    cp_wo = pltpu.make_async_copy(wo_hbm, wo_v, w_sem.at[3])
    cp_wg = pltpu.make_async_copy(wg_hbm, wg_v, w_sem.at[4])
    cp_wu = pltpu.make_async_copy(wu_hbm, wu_v, w_sem.at[5])
    cp_wd = [pltpu.make_async_copy(wd_hbm.at[pl.ds(c * fc, fc)], wd_v.at[pl.ds(c * fc, fc)],
                                   d_sem.at[c]) for c in range(_FC)]

    cp_wq.start()
    cp_x.start()
    cp_wr.start()
    cp_wo.start()

    cp_x.wait()
    x = x_v[...].astype(f32)
    xn = _layernorm(x).astype(bf16)
    cp_wq.wait()
    for i in range(_NPAIR):
        kv_copy(kt_hbm, k_ring, k_sem, i).start()
        kv_copy(vt_hbm, v_ring, v_sem, i).start()
    q = jnp.dot(xn, wq_v[...], preferred_element_type=f32)
    for h in range(_H):
        q_s[h] = q[:, h * _DH:(h + 1) * _DH].astype(bf16)
    cp_wo.wait()

    row = jax.lax.broadcasted_iota(jnp.int32, (_B, _DH), 0)
    scale = _DH ** -0.5

    def body(i, acc):
        h = i // _B
        b = i % _B
        slot = i % _NPAIR
        kv_copy(kt_hbm, k_ring, k_sem, i).wait()
        s = jnp.dot(q_s[h], k_ring[slot], preferred_element_type=f32) * scale

        @pl.when(i + _NPAIR < n)
        def _():
            kv_copy(kt_hbm, k_ring, k_sem, i + _NPAIR).start()

        @pl.when(i == n - 2)
        def _():
            cp_wg.start()

        @pl.when(i == n - 1)
        def _():
            cp_wd[0].start()
            cp_wd[1].start()

        m = jnp.max(s, axis=-1, keepdims=True)
        p = jnp.exp(s - m)
        l = jnp.sum(p, axis=-1, keepdims=True)
        kv_copy(vt_hbm, v_ring, v_sem, i).wait()
        o = jax.lax.dot_general(p.astype(bf16), v_ring[slot], (((1,), (1,)), ((), ())),
                                preferred_element_type=f32)

        @pl.when(i + _NPAIR < n)
        def _():
            kv_copy(vt_hbm, v_ring, v_sem, i + _NPAIR).start()

        @pl.when(i == n - 2)
        def _():
            cp_wu.start()

        @pl.when(i == n - 1)
        def _():
            cp_wd[2].start()
            cp_wd[3].start()

        o = jnp.where(row == b, o / l, 0.0).astype(bf16)
        wo_h = wo_v[pl.ds(pl.multiple_of(h * _DH, 16), _DH), :]
        return acc + jnp.dot(o, wo_h, preferred_element_type=f32)

    attn = jax.lax.fori_loop(0, n, body, jnp.zeros((_B, _D), f32))

    hres = x + attn
    hn = _layernorm(hres)
    hb = hn.astype(bf16)
    cp_wr.wait()
    wr = wr_v[...].astype(f32)
    rp = hn[:, 0:128] * wr[0:1, :]
    for j in range(1, _D // 128):
        rp = rp + hn[:, j * 128:(j + 1) * 128] * wr[j:j + 1, :]
    r = jnp.sum(rp, axis=-1, keepdims=True)
    cp_wg.wait()
    g = jnp.dot(hb, wg_v[...], preferred_element_type=f32)
    cp_wu.wait()
    u = jnp.dot(hb, wu_v[...], preferred_element_type=f32)
    a = (g * jax.nn.sigmoid(g) * u).astype(bf16)
    y = jnp.zeros((_B, _D), f32)
    for c in range(_FC):
        cp_wd[c].wait()
        y = y + jnp.dot(a[:, c * fc:(c + 1) * fc], wd_v[c * fc:(c + 1) * fc, :],
                        preferred_element_type=f32)
    y = y * jax.nn.sigmoid(r)
    o_ref[...] = (hres + (hn + (hn * 0.0 + y))).astype(o_ref.dtype)


@jax.jit
def pallas_sequential_preLN__mha_block_cached__moe_arch_mod__decode_kernel(
    A_x: jax.Array,
    A_k_cache: jax.Array,
    A_v_cache: jax.Array,
    A_wq: jax.Array,
    A_wo: jax.Array,
    B_x: jax.Array,
    B_w_r: jax.Array,
    B_w_gate: jax.Array,
    B_w_up: jax.Array,
    B_w_down: jax.Array,
):
    del B_x
    bf16 = jnp.bfloat16
    hbm = pl.BlockSpec(memory_space=pl.ANY)
    out = pl.pallas_call(
        _kernel,
        out_shape=jax.ShapeDtypeStruct((_B, _D), A_x.dtype),
        in_specs=[hbm] * 9,
        out_specs=pl.BlockSpec(memory_space=pltpu.VMEM),
        scratch_shapes=[
            pltpu.VMEM((_B, _D), bf16),
            pltpu.VMEM((_D, _H * _DH), bf16),
            pltpu.VMEM((_H * _DH, _D), bf16),
            pltpu.VMEM((_D // 128, 128), bf16),
            pltpu.VMEM((_D, _F), bf16),
            pltpu.VMEM((_D, _F), bf16),
            pltpu.VMEM((_F, _D), bf16),
            pltpu.VMEM((_NPAIR, _DH, _S), bf16),
            pltpu.VMEM((_NPAIR, _DH, _S), bf16),
            pltpu.VMEM((_H, _B, _DH), bf16),
            pltpu.SemaphoreType.DMA((_NPAIR,)),
            pltpu.SemaphoreType.DMA((_NPAIR,)),
            pltpu.SemaphoreType.DMA((6,)),
            pltpu.SemaphoreType.DMA((_FC,)),
        ],
        compiler_params=pltpu.CompilerParams(vmem_limit_bytes=100 * 1024 * 1024),
    )(
        A_x.reshape(_B, _D),
        jnp.transpose(A_k_cache, (0, 1, 3, 2)),
        jnp.transpose(A_v_cache, (0, 1, 3, 2)),
        A_wq,
        A_wo,
        B_w_r.reshape(_D // 128, 128),
        B_w_gate,
        B_w_up,
        B_w_down,
    )
    return out.reshape(_B, 1, _D)
```

```python
import jax
import jax.numpy as jnp
import jax.experimental.pallas as pl
import jax.experimental.pallas.tpu as pltpu

_B, _H, _DH, _S, _D, _F = 4, 32, 192, 8192, 640, 1536
_LOOK = 3
_NSLOT = _LOOK + 1
_CB = 512
_DW = 256
_FC = 4
_TAIL = (24, 24, 24)
_EPS = 1e-5


def _layernorm(x):
    m = jnp.mean(x, axis=-1, keepdims=True)
    c = x - m
    v = jnp.mean(c * c, axis=-1, keepdims=True)
    return c / jnp.sqrt(v + _EPS)


def _pieces(src, dst, sem, rows, cols):
    nr, nc = src.shape
    return [pltpu.make_async_copy(src.at[pl.ds(r, rows), pl.ds(c, cols)],
                                  dst.at[pl.ds(r, rows), pl.ds(c, cols)], sem)
            for r in range(0, nr, rows) for c in range(0, nc, cols)]


def _start(copies):
    for j, cp in enumerate(copies):
        cp.start(priority=j % 2)


def _wait_all(buf, sem):
    pltpu.make_async_copy(buf, buf, sem).wait()


def _spread(copies, steps):
    pairs = [copies[j:j + 2] for j in range(0, len(copies), 2)]
    n = len(pairs)
    return [sum(pairs[n * s // steps:n * (s + 1) // steps], []) for s in range(steps)]


def _kernel(x_hbm, kt_hbm, vt_hbm, wq_hbm, wo_hbm, wr_hbm, wg_hbm, wu_hbm, wd_hbm,
            o_ref,
            x_v, wq_v, wo_v, wr_v, wg_v, wu_v, wd_v, k_ring, v_ring, q_s,
            k_sem, v_sem, w_sem, d_sem):
    f32, bf16 = jnp.float32, jnp.bfloat16
    n = _B * _H
    fc = _F // _FC
    nblk = _S // _CB

    def kv_pieces(src, ring, sem, i):
        slot = i % _NSLOT
        return _pieces(src.at[i % _B, i // _B], ring.at[slot], sem.at[slot], _DH, _DW)

    cp_x = pltpu.make_async_copy(x_hbm, x_v, w_sem.at[1])
    cp_wr = pltpu.make_async_copy(wr_hbm, wr_v, w_sem.at[2])
    wq_p = _pieces(wq_hbm, wq_v, w_sem.at[0], 160, 256)
    wo_p = _pieces(wo_hbm, wo_v, w_sem.at[3], 64, _D)

    _start(wq_p[:2])
    cp_x.start()
    cp_wr.start(priority=1)
    _start(wq_p[2:])
    _start(wo_p[:48])

    cp_x.wait()
    x = x_v[...].astype(f32)
    xn = _layernorm(x).astype(bf16)
    _wait_all(wq_v, w_sem.at[0])
    rest = wo_p[48:]
    for i in range(_LOOK):
        rest = rest + kv_pieces(kt_hbm, k_ring, k_sem, i) + kv_pieces(vt_hbm, v_ring, v_sem, i)
    rest = _spread(rest, _H // 2)
    for hp in range(_H // 2):
        _start(rest[hp])
        q = jnp.dot(xn, wq_v[:, hp * 2 * _DH:(hp + 1) * 2 * _DH], preferred_element_type=f32)
        q_s[2 * hp] = q[:, :_DH].astype(bf16)
        q_s[2 * hp + 1] = q[:, _DH:].astype(bf16)
    _wait_all(wo_v, w_sem.at[3])

    row = jax.lax.broadcasted_iota(jnp.int32, (_B, _DH), 0)
    scale = _DH ** -0.5

    def step(i, acc, during_qk, during_pv):
        h = i // _B
        b = i % _B
        slot = i % _NSLOT
        _wait_all(k_ring.at[slot], k_sem.at[slot])
        qh = q_s[h]
        s = []
        for j in range(nblk):
            _start(during_qk[j])
            s.append(jnp.dot(qh, k_ring[slot, :, j * _CB:(j + 1) * _CB],
                             preferred_element_type=f32) * scale)
        mx = s[0]
        for j in range(1, nblk):
            mx = jnp.maximum(mx, s[j])
        m = jnp.max(mx, axis=-1, keepdims=True)
        _wait_all(v_ring.at[slot], v_sem.at[slot])
        o = jnp.zeros((_B, _DH), f32)
        ls = jnp.zeros((_B, _CB), f32)
        for j in range(nblk):
            _start(during_pv[j])
            p = jnp.exp(s[j] - m)
            ls = ls + p
            o = o + jax.lax.dot_general(p.astype(bf16), v_ring[slot, :, j * _CB:(j + 1) * _CB],
                                        (((1,), (1,)), ((), ())), preferred_element_type=f32)
        l = jnp.sum(ls, axis=-1, keepdims=True)
        o = jnp.where(row == b, o / l, 0.0).astype(bf16)
        wo_h = wo_v[pl.ds(pl.multiple_of(h * _DH, 16), _DH), :]
        return acc + jnp.dot(o, wo_h, preferred_element_type=f32)

    def body(i, acc):
        return step(i, acc,
                    _spread(kv_pieces(kt_hbm, k_ring, k_sem, i + _LOOK), nblk),
                    _spread(kv_pieces(vt_hbm, v_ring, v_sem, i + _LOOK), nblk))

    attn = jax.lax.fori_loop(0, n - _LOOK, body, jnp.zeros((_B, _D), f32))

    ffn = _pieces(wg_hbm, wg_v, w_sem.at[4], 160, 256) + _pieces(wu_hbm, wu_v, w_sem.at[5], 160, 256)
    for c in range(_FC):
        ffn = ffn + _pieces(wd_hbm.at[pl.ds(c * fc, fc)], wd_v.at[pl.ds(c * fc, fc)], d_sem.at[c], 64, _D)
    pos = 0
    for t in range(_LOOK):
        sp = _spread(ffn[pos:pos + _TAIL[t]], 2 * nblk)
        pos += _TAIL[t]
        attn = step(n - _LOOK + t, attn, sp[:nblk], sp[nblk:])
    _start(ffn[pos:])

    hres = x + attn
    hn = _layernorm(hres)
    hb = hn.astype(bf16)
    cp_wr.wait()
    wr = wr_v[...].astype(f32)
    rp = hn[:, 0:128] * wr[0:1, :]
    for j in range(1, _D // 128):
        rp = rp + hn[:, j * 128:(j + 1) * 128] * wr[j:j + 1, :]
    r = jnp.sum(rp, axis=-1, keepdims=True)
    _wait_all(wg_v, w_sem.at[4])
    g = jnp.dot(hb, wg_v[...], preferred_element_type=f32)
    _wait_all(wu_v, w_sem.at[5])
    u = jnp.dot(hb, wu_v[...], preferred_element_type=f32)
    a = (g * jax.nn.sigmoid(g) * u).astype(bf16)
    y = jnp.zeros((_B, _D), f32)
    for c in range(_FC):
        _wait_all(wd_v.at[pl.ds(c * fc, fc)], d_sem.at[c])
        y = y + jnp.dot(a[:, c * fc:(c + 1) * fc], wd_v[c * fc:(c + 1) * fc, :],
                        preferred_element_type=f32)
    y = y * jax.nn.sigmoid(r)
    o_ref[...] = (hres + (hn + (hn * 0.0 + y))).astype(o_ref.dtype)


@jax.jit
def pallas_sequential_preLN__mha_block_cached__moe_arch_mod__decode_kernel(
    A_x, A_k_cache, A_v_cache, A_wq, A_wo, B_x, B_w_r, B_w_gate, B_w_up, B_w_down):
    del B_x
    bf16 = jnp.bfloat16
    hbm = pl.BlockSpec(memory_space=pl.ANY)
    out = pl.pallas_call(
        _kernel,
        out_shape=jax.ShapeDtypeStruct((_B, _D), A_x.dtype),
        in_specs=[hbm] * 9,
        out_specs=pl.BlockSpec(memory_space=pltpu.VMEM),
        scratch_shapes=[
            pltpu.VMEM((_B, _D), bf16),
            pltpu.VMEM((_D, _H * _DH), bf16),
            pltpu.VMEM((_H * _DH, _D), bf16),
            pltpu.VMEM((_D // 128, 128), bf16),
            pltpu.VMEM((_D, _F), bf16),
            pltpu.VMEM((_D, _F), bf16),
            pltpu.VMEM((_F, _D), bf16),
            pltpu.VMEM((_NSLOT, _DH, _S), bf16),
            pltpu.VMEM((_NSLOT, _DH, _S), bf16),
            pltpu.VMEM((_H, _B, _DH), bf16),
            pltpu.SemaphoreType.DMA((_NSLOT,)),
            pltpu.SemaphoreType.DMA((_NSLOT,)),
            pltpu.SemaphoreType.DMA((6,)),
            pltpu.SemaphoreType.DMA((_FC,)),
        ],
        compiler_params=pltpu.CompilerParams(vmem_limit_bytes=100 * 1024 * 1024),
    )(
        A_x.reshape(_B, _D),
        jnp.transpose(A_k_cache, (0, 1, 3, 2)),
        jnp.transpose(A_v_cache, (0, 1, 3, 2)),
        A_wq,
        A_wo,
        B_w_r.reshape(_D // 128, 128),
        B_w_gate,
        B_w_up,
        B_w_down,
    )
    return out.reshape(_B, 1, _D)
```

```python
import jax
import jax.numpy as jnp
import jax.experimental.pallas as pl
import jax.experimental.pallas.tpu as pltpu

_B, _H, _DH, _S, _D, _F = 4, 32, 192, 8192, 640, 1536
_P = 2 * _DH
_HP = _H // 2
_LOOK = 2
_NSLOT = _LOOK + 1
_CB = 512
_KV_BANDS = (136, 136, 112)
_FC = 4
_TAIL = (24, 24)
_EPS = 1e-5


def _layernorm(x):
    m = jnp.mean(x, axis=-1, keepdims=True)
    c = x - m
    v = jnp.mean(c * c, axis=-1, keepdims=True)
    return c / jnp.sqrt(v + _EPS)


def _pieces(src, dst, sem, bands, cols):
    nr, nc = src.shape
    out, r, k = [], 0, 0
    while r < nr:
        rows = bands[k % len(bands)]
        out += [pltpu.make_async_copy(src.at[pl.ds(r, rows), pl.ds(c, cols)],
                                      dst.at[pl.ds(r, rows), pl.ds(c, cols)], sem)
                for c in range(0, nc, cols)]
        r, k = r + rows, k + 1
    assert r == nr and nc % cols == 0
    return out


def _start(copies):
    for j, cp in enumerate(copies):
        cp.start(priority=j % 2)


def _wait_all(buf, sem):
    pltpu.make_async_copy(buf, buf, sem).wait()


def _spread(copies, steps):
    pairs = [copies[j:j + 2] for j in range(0, len(copies), 2)]
    n = len(pairs)
    return [sum(pairs[n * s // steps:n * (s + 1) // steps], []) for s in range(steps)]


def _kernel(x_hbm, kt_hbm, vt_hbm, wq_hbm, wo_hbm, wr_hbm, wg_hbm, wu_hbm, wd_hbm,
            o_ref,
            x_v, wq_v, wo_v, wr_v, wg_v, wu_v, wd_v, k_ring, v_ring, q_s,
            k_sem, v_sem, w_sem, d_sem):
    f32, bf16 = jnp.float32, jnp.bfloat16
    n = _B * _HP
    fc = _F // _FC
    nblk = _S // _CB

    def kv_pieces(src, ring, sem, i):
        slot = i % _NSLOT
        return _pieces(src.at[i], ring.at[slot], sem.at[slot], _KV_BANDS, 256)

    cp_x = pltpu.make_async_copy(x_hbm, x_v, w_sem.at[1])
    cp_wr = pltpu.make_async_copy(wr_hbm, wr_v, w_sem.at[2])
    wq_p = _pieces(wq_hbm, wq_v, w_sem.at[0], (160,), 256)
    _start(wq_p[:2])
    _start([cp_x, cp_wr])
    _start(wq_p[2:])
    _start(_pieces(wo_hbm, wo_v, w_sem.at[3], (64,), _D))
    first = []
    for i in range(_LOOK):
        first += kv_pieces(kt_hbm, k_ring, k_sem, i) + kv_pieces(vt_hbm, v_ring, v_sem, i)
    first = _spread(first, _HP)

    row = jax.lax.broadcasted_iota(jnp.int32, (2 * _B, _P), 0)
    col = jax.lax.broadcasted_iota(jnp.int32, (2 * _B, _P), 1)
    own_head = (row < _B) == (col < _DH)

    cp_x.wait()
    x = x_v[...].astype(f32)
    xn = _layernorm(x).astype(bf16)
    xn2 = jnp.concatenate([xn, xn], axis=0)
    _wait_all(wq_v, w_sem.at[0])
    for hp in range(_HP):
        _start(first[hp])
        q = jnp.dot(xn2, wq_v[:, hp * _P:(hp + 1) * _P], preferred_element_type=f32)
        q_s[hp] = jnp.where(own_head, q, 0.0).astype(bf16)
    _wait_all(wo_v, w_sem.at[3])

    ffn = (_pieces(wg_hbm, wg_v, w_sem.at[4], (32,), _F)
           + _pieces(wu_hbm, wu_v, w_sem.at[5], (32,), _F))
    for c in range(_FC):
        ffn += _pieces(wd_hbm.at[pl.ds(c * fc, fc)], wd_v.at[pl.ds(c * fc, fc)],
                       d_sem.at[c], (64,), _D)

    scale = _DH ** -0.5

    def step(i, acc):
        for t in range(_LOOK):
            lo = sum(_TAIL[:t])
            pl.when(i == n - _LOOK + t)(lambda c=ffn[lo:lo + _TAIL[t]]: _start(c))
        more = i + _LOOK < n
        nxt = jnp.minimum(i + _LOOK, n - 1)
        next_k = _spread(kv_pieces(kt_hbm, k_ring, k_sem, nxt), nblk)
        next_v = _spread(kv_pieces(vt_hbm, v_ring, v_sem, nxt), nblk)
        b = i // _HP
        hp = i % _HP
        slot = i % _NSLOT

        _wait_all(k_ring.at[slot], k_sem.at[slot])
        qh = q_s[hp]
        s = []
        for j in range(nblk):
            pl.when(more)(lambda c=next_k[j]: _start(c))
            s.append(jnp.dot(qh, k_ring[slot, :, j * _CB:(j + 1) * _CB],
                             preferred_element_type=f32) * scale)
        mx = s[0]
        for j in range(1, nblk):
            mx = jnp.maximum(mx, s[j])
        m = jnp.max(mx, axis=-1, keepdims=True)

        _wait_all(v_ring.at[slot], v_sem.at[slot])
        o = jnp.zeros((2 * _B, _P), f32)
        ls = jnp.zeros((2 * _B, _CB), f32)
        for j in range(nblk):
            pl.when(more)(lambda c=next_v[j]: _start(c))
            p = jnp.exp(s[j] - m)
            ls = ls + p
            o = o + jax.lax.dot_general(p.astype(bf16), v_ring[slot, :, j * _CB:(j + 1) * _CB],
                                        (((1,), (1,)), ((), ())), preferred_element_type=f32)
        l = jnp.sum(ls, axis=-1, keepdims=True)
        keep = own_head & ((row % _B) == b)
        o = jnp.where(keep, o / l, 0.0).astype(bf16)
        wo_h = wo_v[pl.ds(pl.multiple_of(hp * _P, _P), _P), :]
        return acc + jnp.dot(o, wo_h, preferred_element_type=f32)

    attn = jax.lax.fori_loop(0, n, step, jnp.zeros((2 * _B, _D), f32))
    _start(ffn[sum(_TAIL):])

    h = x + (attn[:_B] + attn[_B:])
    hn = _layernorm(h)
    hb = hn.astype(bf16)
    cp_wr.wait()
    wr = wr_v[...].astype(f32)
    rp = hn[:, 0:128] * wr[0:1, :]
    for j in range(1, _D // 128):
        rp = rp + hn[:, j * 128:(j + 1) * 128] * wr[j:j + 1, :]
    r = jnp.sum(rp, axis=-1, keepdims=True)
    _wait_all(wg_v, w_sem.at[4])
    g = jnp.dot(hb, wg_v[...], preferred_element_type=f32)
    _wait_all(wu_v, w_sem.at[5])
    u = jnp.dot(hb, wu_v[...], preferred_element_type=f32)
    a = (g * jax.nn.sigmoid(g) * u).astype(bf16)
    y = jnp.zeros((_B, _D), f32)
    for c in range(_FC):
        _wait_all(wd_v.at[pl.ds(c * fc, fc)], d_sem.at[c])
        y = y + jnp.dot(a[:, c * fc:(c + 1) * fc], wd_v[c * fc:(c + 1) * fc, :],
                        preferred_element_type=f32)
    y = y * jax.nn.sigmoid(r)
    o_ref[...] = (h + (hn + (hn * 0.0 + y))).astype(o_ref.dtype)


@jax.jit
def pallas_sequential_preLN__mha_block_cached__moe_arch_mod__decode_kernel(
    A_x: jax.Array,
    A_k_cache: jax.Array,
    A_v_cache: jax.Array,
    A_wq: jax.Array,
    A_wo: jax.Array,
    B_x: jax.Array,
    B_w_r: jax.Array,
    B_w_gate: jax.Array,
    B_w_up: jax.Array,
    B_w_down: jax.Array,
):
    del B_x
    bf16 = jnp.bfloat16
    out = pl.pallas_call(
        _kernel,
        out_shape=jax.ShapeDtypeStruct((_B, _D), A_x.dtype),
        in_specs=[pl.BlockSpec(memory_space=pl.ANY)] * 9,
        out_specs=pl.BlockSpec(memory_space=pltpu.VMEM),
        scratch_shapes=[
            pltpu.VMEM((_B, _D), bf16),
            pltpu.VMEM((_D, _H * _DH), bf16),
            pltpu.VMEM((_H * _DH, _D), bf16),
            pltpu.VMEM((_D // 128, 128), bf16),
            pltpu.VMEM((_D, _F), bf16),
            pltpu.VMEM((_D, _F), bf16),
            pltpu.VMEM((_F, _D), bf16),
            pltpu.VMEM((_NSLOT, _P, _S), bf16),
            pltpu.VMEM((_NSLOT, _P, _S), bf16),
            pltpu.VMEM((_HP, 2 * _B, _P), bf16),
            pltpu.SemaphoreType.DMA((_NSLOT,)),
            pltpu.SemaphoreType.DMA((_NSLOT,)),
            pltpu.SemaphoreType.DMA((6,)),
            pltpu.SemaphoreType.DMA((_FC,)),
        ],
        compiler_params=pltpu.CompilerParams(vmem_limit_bytes=100 * 1024 * 1024),
    )(
        A_x.reshape(_B, _D),
        jnp.transpose(A_k_cache, (0, 1, 3, 2)).reshape(_B * _HP, _P, _S),
        jnp.transpose(A_v_cache, (0, 1, 3, 2)).reshape(_B * _HP, _P, _S),
        A_wq,
        A_wo,
        B_w_r.reshape(_D // 128, 128),
        B_w_gate,
        B_w_up,
        B_w_down,
    )
    return out.reshape(_B, 1, _D)
```
